```python
import os as _os
_os.environ.setdefault("JAX_PLATFORMS", "cpu")
import jax
import jax.numpy as jnp

def _softmax(x, axis=-1):
    return jax.nn.softmax(x, axis=axis)
def _gelu(x):
    return jax.nn.gelu(x, approximate=True)
def _silu(x):
    return jax.nn.silu(x)
def _sigmoid(x):
    return jax.nn.sigmoid(x)
def _layernorm(x, axis=-1, eps=1e-5):
    m = jnp.mean(x, axis=axis, keepdims=True)
    v = jnp.var(x, axis=axis, keepdims=True)
    return (x - m) / jnp.sqrt(v + eps)
def _scatter_add(tgt, idx, src, axis=0):
    return tgt.at[idx].add(src)
def _segment_sum(src, seg, n):
    return jax.ops.segment_sum(src, seg, n)
class _Rng:
    def __init__(self, key):
        self._k = key
    def _next(self):
        self._k, sub = jax.random.split(self._k)
        return sub
    def normal(self, shape):
        return jax.random.normal(self._next(), shape, dtype=jnp.bfloat16)
    def randint(self, lo, hi, shape):
        return jax.random.randint(self._next(), shape, lo, hi, dtype=jnp.int32)
    def uniform(self, shape, lo=0.0, hi=1.0):
        return jax.random.uniform(self._next(), shape, jnp.bfloat16, lo, hi)
    def permutation(self, n):
        return jax.random.permutation(self._next(), n)


kernel_name = 'gated_mix__linear_attn_block__mixer_token_mlp__prompt'

def setup_inputs():
    _rng = _Rng(jax.random.key(int.from_bytes(__import__("os").urandom(4), "little")))
    _w = (lambda a: (lambda t: t.astype(jnp.bfloat16) if jnp.issubdtype(t.dtype, jnp.floating) else t)(jnp.asarray(a)))
    def _A_setup():
        B, S, D = 1, 2048, 512
        return {
            "x": _w((lambda *s: _rng.normal(s) * 0.05)(B, S, D)),
            "wqkv": _w((lambda *s: _rng.normal(s) * 0.8)(D, 3 * D)),
            "wo": _w((lambda *s: _rng.normal(s) * 0.05)(D, D)),
        }
    _A_in = _A_setup()

    def _B_setup():
        B, S, D, F = 1, 2048, 512, 1792
        return {
            "x": _w((lambda *s: _rng.normal(s) * 0.05)(B, S, D)),
            "w1": _w((lambda *s: _rng.normal(s) * 0.1)(S, F) * (S ** -0.5)),
            "b1": _w((lambda *s: _rng.normal(s) * 0.1)(F) * 0.02),
            "w2": _w((lambda *s: _rng.normal(s) * 0.1)(F, S) * (F ** -0.5)),
            "b2": _w((lambda *s: _rng.normal(s) * 0.1)(S) * 0.02),
        }
    _B_in = _B_setup()

    return {
        "A_x": _A_in["x"],
        "A_wqkv": _A_in["wqkv"],
        "A_wo": _A_in["wo"],
        "B_x": _B_in["x"],
        "B_w1": _B_in["w1"],
        "B_b1": _B_in["b1"],
        "B_w2": _B_in["w2"],
        "B_b2": _B_in["b2"],
        "gate_w": _w((lambda *s: _rng.normal(s) * 0.05)(512) * 16.0),
    }

def reference(A_x, A_wqkv, A_wo, B_x, B_w1, B_b1, B_w2, B_b2, gate_w):
    def _A_ref(x, wqkv, wo):
        B, S, D = x.shape
        H = 32; Dh = D // H
        qkv = (lambda x, *d: x.transpose(*d))((x @ wqkv).reshape(B, S, 3, H, Dh), 2, 0, 3, 1, 4)
        q, k, v = qkv[0], qkv[1], qkv[2]
        phi = lambda t: jnp.where(t > 0, t + 1, jnp.exp(t)) + 1e-6
        pq, pk = phi(q), phi(k)
        kv = jnp.einsum("bhsd,bhse->bhde", pk, v)
        z = jnp.einsum("bhsd->bhd", pk)
        num = jnp.einsum("bhqd,bhde->bhqe", pq, kv)
        den = jnp.einsum("bhqd,bhd->bhq", pq, z)[..., None] + 1e-6
        o = num / den
        return (lambda x, *d: x.transpose(*d))(o, 0, 2, 1, 3).reshape(B, S, D) @ wo

    def _B_ref(x, w1, b1, w2, b2):
        B, S, D = x.shape
        h = _layernorm(x, axis=-1)
        u = jnp.einsum("bsd,sf->bdf", h, w1) + b1
        u = _gelu(u)
        y = jnp.einsum("bdf,fs->bds", u, w2) + b2
        return (lambda x, *d: x.transpose(*d))(y, 0, 2, 1)

    x = A_x
    g = _sigmoid((x * gate_w).sum(-1, keepdims=True))
    a = _A_ref(x, A_wqkv, A_wo)
    b = _B_ref(x, B_w1, B_b1, B_w2, B_b2)
    return g * a + (1 - g) * b
```

```python
import jax
import jax.numpy as jnp
from jax import lax
import jax.experimental.pallas as pl
import jax.experimental.pallas.tpu as pltpu

_F32 = jnp.float32
_BF16 = jnp.bfloat16
_LANE = 128


def _phi(t):
    return jnp.where(t > 0, t + 1.0, jnp.exp(t)) + 1e-6


def _dot(a, b):
    return jnp.dot(a, b, preferred_element_type=_F32)


def _make_kernel(S, D, F, H, TS):
    NT = S // TS
    DH = D // H
    NJ = D // _LANE

    def kernel(x_hbm, wqkv_hbm, wo_hbm, w1_hbm, w2_hbm, b1_ref, b2_ref, gw_ref,
               out_hbm,
               x_v, wqkv_v, wo_v, w1_v, w2_v, out_v, pq_s, hT_s,
               in_sems, out_sems):
        def x_copy(t):
            return pltpu.make_async_copy(
                x_hbm.at[pl.ds(t * TS, TS), :], x_v.at[pl.ds(t * TS, TS), :],
                in_sems.at[t])

        def w1_copy(t):
            return pltpu.make_async_copy(
                w1_hbm.at[pl.ds(t * TS, TS), :], w1_v.at[pl.ds(t * TS, TS), :],
                in_sems.at[NT + t])

        wqkv_copy = pltpu.make_async_copy(wqkv_hbm, wqkv_v, in_sems.at[2 * NT])
        wo_copy = pltpu.make_async_copy(wo_hbm, wo_v, in_sems.at[2 * NT + 1])
        w2_copy = pltpu.make_async_copy(w2_hbm, w2_v, in_sems.at[2 * NT + 2])

        def out_copy(t):
            return pltpu.make_async_copy(
                out_v.at[pl.ds(t * TS, TS), :], out_hbm.at[pl.ds(t * TS, TS), :],
                out_sems.at[t])

        x_copy(0).start()
        wqkv_copy.start()
        for t in range(1, NT):
            x_copy(t).start()
            w1_copy(t - 1).start()
        w1_copy(NT - 1).start()
        wo_copy.start()
        w2_copy.start()

        wqkv_copy.wait()
        wkT = wqkv_v[:, D:2 * D].astype(_F32).T.astype(_BF16)
        wq = wqkv_v[:, 0:D]
        wv = wqkv_v[:, 2 * D:3 * D]

        kv_acc = [None] * NJ
        z_acc = None
        for t in range(NT):
            x_copy(t).wait()
            xt = x_v[t * TS:(t + 1) * TS, :]
            xT = xt.astype(_F32).T
            mu = jnp.mean(xT, axis=0, keepdims=True)
            xc = xT - mu
            var = jnp.mean(xc * xc, axis=0, keepdims=True)
            hT_s[:, t * TS:(t + 1) * TS] = (
                xc * lax.rsqrt(var + 1e-5)).astype(_BF16)

            pkT = _phi(_dot(wkT, xT.astype(_BF16)))
            zt = jnp.sum(pkT, axis=1, keepdims=True)
            z_acc = zt if z_acc is None else z_acc + zt
            pkT = pkT.astype(_BF16)

            pq_s[t * TS:(t + 1) * TS, :] = _phi(_dot(xt, wq)).astype(_BF16)
            v = _dot(xt, wv).astype(_BF16)
            for j in range(NJ):
                sl = slice(j * _LANE, (j + 1) * _LANE)
                kvj = _dot(pkT[sl, :], v[:, sl])
                kv_acc[j] = kvj if kv_acc[j] is None else kv_acc[j] + kvj

        rowh = lax.broadcasted_iota(jnp.int32, (_LANE, _LANE), 0) // DH
        colh = lax.broadcasted_iota(jnp.int32, (_LANE, _LANE), 1) // DH
        same = rowh == colh
        kvz = []
        for j in range(NJ):
            zj = jnp.broadcast_to(z_acc[j * _LANE:(j + 1) * _LANE, :],
                                  (_LANE, _LANE))
            kvz.append(jnp.concatenate(
                [jnp.where(same, kv_acc[j], 0.0), jnp.where(same, zj, 0.0)],
                axis=1).astype(_BF16))

        for t in range(NT):
            w1_copy(t).wait()
        u = _dot(hT_s[...], w1_v[...]) + b1_ref[...].astype(_F32)
        u = jax.nn.gelu(u, approximate=True).astype(_BF16)

        wo_copy.wait()
        w2_copy.wait()
        gw = gw_ref[...].astype(_F32)

        for t in range(NT):
            rows = slice(t * TS, (t + 1) * TS)
            pq = pq_s[rows, :]
            a = None
            for j in range(NJ):
                sl = slice(j * _LANE, (j + 1) * _LANE)
                nd = _dot(pq[:, sl], kvz[j])
                oj = (nd[:, :_LANE] / (nd[:, _LANE:] + 1e-6)).astype(_BF16)
                aj = _dot(oj, wo_v[sl, :])
                a = aj if a is None else a + aj
            y = _dot(u, w2_v[:, rows]) + b2_ref[:, rows].astype(_F32)
            yT = y.T
            xt = x_v[rows, :].astype(_F32)
            g = jax.nn.sigmoid(jnp.sum(xt * gw, axis=-1, keepdims=True))
            out_v[rows, :] = (g * a + (1.0 - g) * yT).astype(_BF16)
            out_copy(t).start()
        for t in range(NT):
            out_copy(t).wait()

    return kernel


@jax.jit
def pallas_gated_mix__linear_attn_block__mixer_token_mlp__prompt_kernel(
    A_x: jax.Array,
    A_wqkv: jax.Array,
    A_wo: jax.Array,
    B_x: jax.Array,
    B_w1: jax.Array,
    B_b1: jax.Array,
    B_w2: jax.Array,
    B_b2: jax.Array,
    gate_w: jax.Array,
):
    B, S, D = A_x.shape
    assert B == 1
    F = B_w1.shape[1]
    H = 32
    TS = 512
    assert S % TS == 0 and D % _LANE == 0 and _LANE % (D // H) == 0

    x2 = A_x.reshape(S, D)
    b1 = B_b1.reshape(1, F)
    b2 = B_b2.reshape(1, S)
    gw = gate_w.reshape(1, D)

    kernel = _make_kernel(S, D, F, H, TS)
    NT = S // TS
    hbm = pl.BlockSpec(memory_space=pl.ANY)
    vmem = pl.BlockSpec(memory_space=pltpu.VMEM)
    out = pl.pallas_call(
        kernel,
        out_shape=jax.ShapeDtypeStruct((S, D), A_x.dtype),
        in_specs=[hbm, hbm, hbm, hbm, hbm, vmem, vmem, vmem],
        out_specs=hbm,
        scratch_shapes=[
            pltpu.VMEM((S, D), _BF16),
            pltpu.VMEM((D, 3 * D), _BF16),
            pltpu.VMEM((D, D), _BF16),
            pltpu.VMEM((S, F), _BF16),
            pltpu.VMEM((F, S), _BF16),
            pltpu.VMEM((S, D), _BF16),
            pltpu.VMEM((S, D), _BF16),
            pltpu.VMEM((D, S), _BF16),
            pltpu.SemaphoreType.DMA((2 * NT + 3,)),
            pltpu.SemaphoreType.DMA((NT,)),
        ],
        compiler_params=pltpu.CompilerParams(
            vmem_limit_bytes=100 * 1024 * 1024),
    )(x2, A_wqkv, A_wo, B_w1, B_w2, b1, b2, gw)
    return out.reshape(B, S, D)
```

```python
import jax
import jax.numpy as jnp
from jax import lax
import jax.experimental.pallas as pl
import jax.experimental.pallas.tpu as pltpu

_F32 = jnp.float32
_BF16 = jnp.bfloat16
_LANE = 128


def _phi(t):
    return jnp.where(t > 0, t + 1.0, jnp.exp(t)) + 1e-6


def _dot(a, b):
    return jnp.dot(a, b, preferred_element_type=_F32)


def _ranges(sizes):
    out, s = [], 0
    for n in sizes:
        out.append((s, n))
        s += n
    return out


def _make_kernel(S, D, F, H, a_tiles, b_tiles):
    DH = D // H
    NJ = D // _LANE
    A = _ranges(a_tiles)
    Bt = _ranges(b_tiles)
    NA, NB = len(A), len(Bt)

    def kernel(x_hbm, wqkv_hbm, wo_hbm, w1_hbm, w2_hbm, b1_ref, b2_ref, gw_ref,
               out_hbm,
               x_v, wqkv_v, wo_v, w1_v, w2_v, out_v, pq_s, hT_s,
               in_sems, out_sems):
        def x_copy(t):
            s, n = A[t]
            return pltpu.make_async_copy(
                x_hbm.at[pl.ds(s, n), :], x_v.at[pl.ds(s, n), :], in_sems.at[t])

        def w1_copy(t):
            s, n = A[t]
            return pltpu.make_async_copy(
                w1_hbm.at[pl.ds(s, n), :], w1_v.at[pl.ds(s, n), :],
                in_sems.at[NA + t])

        def wqkv_copy(i):
            return pltpu.make_async_copy(
                wqkv_hbm.at[:, pl.ds(i * D, D)], wqkv_v.at[:, pl.ds(i * D, D)],
                in_sems.at[2 * NA + i])

        wo_copy = pltpu.make_async_copy(wo_hbm, wo_v, in_sems.at[2 * NA + 4])
        w2_copy = pltpu.make_async_copy(w2_hbm, w2_v, in_sems.at[2 * NA + 5])

        def out_copy(t):
            s, n = Bt[t]
            return pltpu.make_async_copy(
                out_v.at[pl.ds(s, n), :], out_hbm.at[pl.ds(s, n), :],
                out_sems.at[t])

        x_copy(0).start()
        for i in range(3):
            wqkv_copy(i).start()
        for t in range(1, NA):
            x_copy(t).start()
            w1_copy(t - 1).start()
        w1_copy(NA - 1).start()
        wo_copy.start()
        w2_copy.start()

        kv_acc = [None] * NJ
        z_acc = None
        wq = wkT = wv = None
        for t in range(NA):
            s, n = A[t]
            x_copy(t).wait()
            xt = x_v[s:s + n, :]
            xT = xt.astype(_F32).T
            mu = jnp.mean(xT, axis=0, keepdims=True)
            xc = xT - mu
            var = jnp.mean(xc * xc, axis=0, keepdims=True)
            hT_s[:, s:s + n] = (xc * lax.rsqrt(var + 1e-5)).astype(_BF16)

            if t == 0:
                wqkv_copy(0).wait()
                wq = wqkv_v[:, 0:D]
            pq_s[s:s + n, :] = _phi(_dot(xt, wq)).astype(_BF16)

            if t == 0:
                wqkv_copy(1).wait()
                wkT = wqkv_v[:, D:2 * D].astype(_F32).T.astype(_BF16)
            pkT = _phi(_dot(wkT, xT.astype(_BF16)))
            zt = jnp.sum(pkT, axis=1, keepdims=True)
            z_acc = zt if z_acc is None else z_acc + zt
            pkT = pkT.astype(_BF16)

            if t == 0:
                wqkv_copy(2).wait()
                wv = wqkv_v[:, 2 * D:3 * D]
            v = _dot(xt, wv).astype(_BF16)
            for j in range(NJ):
                sl = slice(j * _LANE, (j + 1) * _LANE)
                kvj = _dot(pkT[sl, :], v[:, sl])
                kv_acc[j] = kvj if kv_acc[j] is None else kv_acc[j] + kvj

        rowh = lax.broadcasted_iota(jnp.int32, (_LANE, _LANE), 0) // DH
        colh = lax.broadcasted_iota(jnp.int32, (_LANE, _LANE), 1) // DH
        same = rowh == colh
        kvz = []
        for j in range(NJ):
            zj = jnp.broadcast_to(z_acc[j * _LANE:(j + 1) * _LANE, :],
                                  (_LANE, _LANE))
            kvz.append(jnp.concatenate(
                [jnp.where(same, kv_acc[j], 0.0), jnp.where(same, zj, 0.0)],
                axis=1).astype(_BF16))

        for t in range(NA):
            w1_copy(t).wait()
        u = _dot(hT_s[...], w1_v[...]) + b1_ref[...].astype(_F32).reshape(1, F)
        u = jax.nn.gelu(u, approximate=True).astype(_BF16)

        wo_copy.wait()
        w2_copy.wait()
        gw = gw_ref[...].astype(_F32).reshape(1, D)
        b2 = b2_ref[...].astype(_F32).reshape(1, S)

        for t in range(NB):
            s, n = Bt[t]
            rows = slice(s, s + n)
            pq = pq_s[rows, :]
            a = None
            for j in range(NJ):
                sl = slice(j * _LANE, (j + 1) * _LANE)
                nd = _dot(pq[:, sl], kvz[j])
                oj = (nd[:, :_LANE] / (nd[:, _LANE:] + 1e-6)).astype(_BF16)
                aj = _dot(oj, wo_v[sl, :])
                a = aj if a is None else a + aj
            y = _dot(u, w2_v[:, rows]) + b2[:, rows]
            yT = y.T
            xt = x_v[rows, :].astype(_F32)
            g = jax.nn.sigmoid(jnp.sum(xt * gw, axis=-1, keepdims=True))
            out_v[rows, :] = (g * a + (1.0 - g) * yT).astype(_BF16)
            out_copy(t).start()
        for t in range(NB):
            out_copy(t).wait()

    return kernel, NA, NB


_A_TILES = (512, 512, 512, 512)
_B_TILES = (512, 512, 512, 256, 256)


@jax.jit
def pallas_gated_mix__linear_attn_block__mixer_token_mlp__prompt_kernel(
    A_x: jax.Array,
    A_wqkv: jax.Array,
    A_wo: jax.Array,
    B_x: jax.Array,
    B_w1: jax.Array,
    B_b1: jax.Array,
    B_w2: jax.Array,
    B_b2: jax.Array,
    gate_w: jax.Array,
):
    B, S, D = A_x.shape
    assert B == 1
    F = B_w1.shape[1]
    H = 32
    assert sum(_A_TILES) == S and sum(_B_TILES) == S
    assert D % _LANE == 0 and _LANE % (D // H) == 0

    x2 = A_x.reshape(S, D)
    kernel, NA, NB = _make_kernel(S, D, F, H, _A_TILES, _B_TILES)
    hbm = pl.BlockSpec(memory_space=pl.ANY)
    vmem = pl.BlockSpec(memory_space=pltpu.VMEM)
    out = pl.pallas_call(
        kernel,
        out_shape=jax.ShapeDtypeStruct((S, D), A_x.dtype),
        in_specs=[hbm, hbm, hbm, hbm, hbm, vmem, vmem, vmem],
        out_specs=hbm,
        scratch_shapes=[
            pltpu.VMEM((S, D), _BF16),
            pltpu.VMEM((D, 3 * D), _BF16),
            pltpu.VMEM((D, D), _BF16),
            pltpu.VMEM((S, F), _BF16),
            pltpu.VMEM((F, S), _BF16),
            pltpu.VMEM((S, D), _BF16),
            pltpu.VMEM((S, D), _BF16),
            pltpu.VMEM((D, S), _BF16),
            pltpu.SemaphoreType.DMA((2 * NA + 6,)),
            pltpu.SemaphoreType.DMA((NB,)),
        ],
        compiler_params=pltpu.CompilerParams(
            vmem_limit_bytes=100 * 1024 * 1024),
    )(x2, A_wqkv, A_wo, B_w1, B_w2, B_b1, B_b2, gate_w)
    return out.reshape(B, S, D)
```
